```python
import os as _os
_os.environ.setdefault("JAX_PLATFORMS", "cpu")
import jax
import jax.numpy as jnp

def _softmax(x, axis=-1):
    return jax.nn.softmax(x, axis=axis)
def _gelu(x):
    return jax.nn.gelu(x, approximate=True)
def _silu(x):
    return jax.nn.silu(x)
def _sigmoid(x):
    return jax.nn.sigmoid(x)
def _layernorm(x, axis=-1, eps=1e-5):
    m = jnp.mean(x, axis=axis, keepdims=True)
    v = jnp.var(x, axis=axis, keepdims=True)
    return (x - m) / jnp.sqrt(v + eps)
def _scatter_add(tgt, idx, src, axis=0):
    return tgt.at[idx].add(src)
def _segment_sum(src, seg, n):
    return jax.ops.segment_sum(src, seg, n)
class _Rng:
    def __init__(self, key):
        self._k = key
    def _next(self):
        self._k, sub = jax.random.split(self._k)
        return sub
    def normal(self, shape):
        return jax.random.normal(self._next(), shape, dtype=jnp.bfloat16)
    def randint(self, lo, hi, shape):
        return jax.random.randint(self._next(), shape, lo, hi, dtype=jnp.int32)
    def uniform(self, shape, lo=0.0, hi=1.0):
        return jax.random.uniform(self._next(), shape, jnp.bfloat16, lo, hi)
    def permutation(self, n):
        return jax.random.permutation(self._next(), n)


kernel_name = 'sequential_preLN__sliding_block_cached__mixer_channel_mlp__decode'

def setup_inputs():
    _rng = _Rng(jax.random.key(int.from_bytes(__import__("os").urandom(4), "little")))
    _w = (lambda a: (lambda t: t.astype(jnp.bfloat16) if jnp.issubdtype(t.dtype, jnp.floating) else t)(jnp.asarray(a)))
    def _A_setup():
        B, Sq, D = 1, 1, 512
        Hq, Hkv, Sk, Dh = 32, 8, 65536, 128
        assert Hq % Hkv == 0, (Hq, Hkv)
        return {
            "x": _w((lambda *s: _rng.normal(s) * 0.05)(B, Sq, D)),
            "k_cache": _w((lambda *s: _rng.normal(s) * 3.2)(B, Hkv, Sk, Dh)),
            "v_cache": _w((lambda *s: _rng.normal(s) * 0.2)(B, Hkv, Sk, Dh)),
            "wq": _w((lambda *s: _rng.normal(s) * 3.2)(D, Hq * Dh) * (D ** -0.5)),
            "wo": _w((lambda *s: _rng.normal(s) * 0.2)(Hq * Dh, D) * ((Hq * Dh) ** -0.5)),
        }
    _A_in = _A_setup()

    def _B_setup():
        B, S, D, F = 1, 1, 512, 1792
        return {
            "x": _w((lambda *s: _rng.normal(s) * 0.05)(B, S, D)),
            "w1": _w((lambda *s: _rng.normal(s) * 0.2)(D, F) * (D ** -0.5)),
            "b1": _w((lambda *s: _rng.normal(s) * 0.2)(F)),
            "w2": _w((lambda *s: _rng.normal(s) * 0.2)(F, D) * (F ** -0.5)),
            "b2": _w((lambda *s: _rng.normal(s) * 0.05)(D)),
        }
    _B_in = _B_setup()

    return {
        "A_x": _A_in["x"],
        "A_k_cache": _A_in["k_cache"],
        "A_v_cache": _A_in["v_cache"],
        "A_wq": _A_in["wq"],
        "A_wo": _A_in["wo"],
        "B_x": _B_in["x"],
        "B_w1": _B_in["w1"],
        "B_b1": _B_in["b1"],
        "B_w2": _B_in["w2"],
        "B_b2": _B_in["b2"],
    }

def reference(A_x, A_k_cache, A_v_cache, A_wq, A_wo, B_x, B_w1, B_b1, B_w2, B_b2):
    def _A_ref(x, k_cache, v_cache, wq, wo):
        B, Sq, D = x.shape
        Hq, Dh = 32, 128
        Hkv, Sk = k_cache.shape[1], k_cache.shape[2]
        W = min(4096, max(256, Sk // 4))
        rep = Hq // Hkv
        q = (lambda x, *d: x.transpose(*d))((x @ wq).reshape(B, Sq, Hq, Dh), 0, 2, 1, 3)
        k = jnp.repeat(k_cache[:, :, Sk - W:, :], rep, axis=1)
        v = jnp.repeat(v_cache[:, :, Sk - W:, :], rep, axis=1)
        scores = jnp.einsum("bhqd,bhkd->bhqk", q, k) * (Dh ** -0.5)
        p = _softmax(scores, axis=-1)
        o = jnp.einsum("bhqk,bhkd->bhqd", p, v)
        return (lambda x, *d: x.transpose(*d))(o, 0, 2, 1, 3).reshape(B, Sq, Hq * Dh) @ wo

    def _B_ref(x, w1, b1, w2, b2):
        y = _layernorm(x, axis=-1)
        h = _gelu(jnp.einsum("bsd,df->bsf", y, w1) + b1)
        return jnp.einsum("bsf,fd->bsd", h, w2) + b2

    x = A_x
    h = x + _A_ref(_layernorm(x, axis=-1), A_k_cache, A_v_cache, A_wq, A_wo)
    h2 = h + _B_ref(_layernorm(h, axis=-1), B_w1, B_b1, B_w2, B_b2)
    return h2
```

```python
import jax, jax.numpy as jnp
from jax import lax
from jax.experimental import pallas as pl
from jax.experimental.pallas import tpu as pltpu

F32, BF16 = jnp.float32, jnp.bfloat16
HQ, DH = 32, 128

def _ln(x):
    m = jnp.mean(x, axis=-1, keepdims=True)
    c = x - m
    v = jnp.mean(c * c, axis=-1, keepdims=True)
    return c * lax.rsqrt(v + 1e-5)

def make(name="k_v1", nodma=False):
    def fn(x, k, v, wq, wo, bx, w1, b1, w2, b2):
        _, hkv, sk, dh = k.shape
        d = x.shape[-1]; f = w1.shape[1]
        win = min(4096, max(256, sk // 4)); s0 = sk - win
        def kern(x_h, k_h, v_h, wq_h, wo_h, w1_h, b1_h, w2_h, b2_h, o_ref,
                 xb, kb, vb, wqb, wob, w1b, b1b, w2b, b2b, sems):
            cp = lambda s, t, i: pltpu.make_async_copy(s, t, sems.at[i])
            c_x = cp(x_h, xb, 0); c_wq = cp(wq_h, wqb, 1)
            c_k = [cp(k_h.at[0, pl.ds(2 * a, 2), pl.ds(s0, win)], kb.at[pl.ds(2 * a, 2)], 2 + a) for a in range(4)]
            c_v = [cp(v_h.at[0, pl.ds(2 * a, 2), pl.ds(s0, win)], vb.at[pl.ds(2 * a, 2)], 6 + a) for a in range(4)]
            c_wo = [cp(wo_h.at[pl.ds(1024 * a, 1024)], wob.at[pl.ds(1024 * a, 1024)], 10 + a) for a in range(4)]
            c_b1 = cp(b1_h, b1b, 14); c_b2 = cp(b2_h, b2b, 15); c_w1 = cp(w1_h, w1b, 16)
            cuts = [0, 1024, 1536, 1664, 1792]
            c_w2 = [cp(w2_h.at[pl.ds(a, b - a)], w2b.at[pl.ds(a, b - a)], 17 + i) for i, (a, b) in enumerate(zip(cuts, cuts[1:]))]
            allc = [c_x, c_wq] + c_k + c_v + c_wo + [c_b1, c_b2, c_w1] + c_w2
            if nodma:
                class N:
                    def wait(self): pass
                for c in allc: c._used = True
                c_x = c_wq = c_b1 = c_b2 = c_w1 = N(); c_k = c_v = c_wo = c_w2 = [N()] * 4
            else:
                for c in allc: c.start()
            c_x.wait()
            x8 = jnp.broadcast_to(xb[0].astype(F32), (8, d))
            xn = _ln(x8).astype(BF16)
            c_wq.wait()
            q = jnp.dot(xn, wqb[...], preferred_element_type=F32)
            row = lax.broadcasted_iota(jnp.int32, (8, dh), 0)
            nt = (((1,), (1,)), ((), ()))
            ps = []
            for a in range(4):
                qa = q[:, 1024 * a:1024 * a + dh]
                for r in range(1, 8):
                    qa = jnp.where(row == r, q[:, 1024 * a + r * dh:1024 * a + (r + 1) * dh], qa)
                qa = qa.astype(BF16)
                c_k[a].wait()
                s_lo = lax.dot_general(qa, kb[2 * a], nt, preferred_element_type=F32)
                s_hi = lax.dot_general(qa, kb[2 * a + 1], nt, preferred_element_type=F32)
                s = jnp.where(row[:, :1] < 4, s_lo, s_hi) * (dh ** -0.5)
                e = jnp.exp(s - jnp.max(s, axis=-1, keepdims=True))
                ps.append((e.astype(BF16), 1.0 / jnp.sum(e, axis=-1, keepdims=True)))
            os_ = []
            for a in range(4):
                e, rl = ps[a]
                c_v[a].wait()
                o_lo = jnp.dot(e, vb[2 * a], preferred_element_type=F32)
                o_hi = jnp.dot(e, vb[2 * a + 1], preferred_element_type=F32)
                os_.append(jnp.where(row < 4, o_lo, o_hi) * rl)
            acc = jnp.zeros((8, d), F32)
            for a in range(4):
                lhs = jnp.concatenate([jnp.where(row == r, os_[a], 0.0) for r in range(8)], axis=1).astype(BF16)
                c_wo[a].wait()
                acc = acc + jnp.dot(lhs, wob[pl.ds(1024 * a, 1024), :], preferred_element_type=F32)
            h = x8 + jnp.sum(acc, axis=0, keepdims=True)
            y = _ln(_ln(h)).astype(BF16)
            c_b1.wait(); c_b2.wait(); c_w1.wait()
            z = jnp.dot(y, w1b[...], preferred_element_type=F32) + b1b[...].astype(F32).reshape(1, f)
            g = jax.nn.gelu(z, approximate=True).astype(BF16)
            out = h + b2b[...].astype(F32).reshape(1, d)
            for i, (a, b) in enumerate(zip(cuts, cuts[1:])):
                c_w2[i].wait()
                out = out + jnp.dot(g[:, a:b], w2b[pl.ds(a, b - a), :], preferred_element_type=F32)
            o_ref[0] = out[0:1].astype(o_ref.dtype)
        hbm = pl.BlockSpec(memory_space=pltpu.HBM)
        V = pltpu.VMEM
        return pl.pallas_call(
            kern, out_shape=jax.ShapeDtypeStruct(x.shape, x.dtype), in_specs=[hbm] * 9,
            scratch_shapes=[V(x.shape, x.dtype), V((hkv, win, dh), k.dtype), V((hkv, win, dh), v.dtype), V(wq.shape, wq.dtype),
                            V(wo.shape, wo.dtype), V(w1.shape, w1.dtype), V(b1.shape, b1.dtype), V(w2.shape, w2.dtype),
                            V(b2.shape, b2.dtype), pltpu.SemaphoreType.DMA((21,))],
            compiler_params=pltpu.CompilerParams(vmem_limit_bytes=48 * 2**20, disable_bounds_checks=True, disable_semaphore_checks=True),
            name=name)(x, k, v, wq, wo, w1, b1, w2, b2)
    return fn


_fn = make("decode_block")


@jax.jit
def pallas_sequential_preLN__sliding_block_cached__mixer_channel_mlp__decode_kernel(
    A_x, A_k_cache, A_v_cache, A_wq, A_wo, B_x, B_w1, B_b1, B_w2, B_b2):
    return _fn(A_x, A_k_cache, A_v_cache, A_wq, A_wo, B_x, B_w1, B_b1, B_w2, B_b2)
```

```python
import numpy as np
import jax, jax.numpy as jnp
from jax import lax
from jax.experimental import pallas as pl
from jax.experimental.pallas import tpu as pltpu

F32, BF16 = jnp.float32, jnp.bfloat16

def _ln(x):
    n = x.shape[-1]
    c = x - jnp.sum(x, axis=-1, keepdims=True) * (1.0 / n)
    v = jnp.sum(c * c, axis=-1, keepdims=True) * (1.0 / n)
    return c * lax.rsqrt(v + 1e-5)

def grp(t, start, visit=None):
    if t in "kv":
        return [(start + j, [(t, 64 * s + j) for s in (visit or range(8))]) for j in range(64)]
    tot = dict(wq=256, wo=256, w1=112, w2=112)[t]
    return [(start + j, [(t, s * 32 + j) for s in (visit or range(8)) if s * 32 + j < tot]) for j in range(32)]

def build_order(*gs):
    rounds = {}
    for g in gs:
        for r, xs in g: rounds.setdefault(r, []).append(xs)
    return [x for r in sorted(rounds) for xs in rounds[r] for x in xs]

blk = lambda *bs: [8 * b + j for b in bs for j in range(8)]
def with_tail(order, stages, ntail):
    tail = stages[len(stages) - ntail:]
    tp = {("w2", p) for bl in tail for p in bl}
    out = [x for x in order if x not in tp]
    for bl in tail:
        out += [("w2", p) for p in sorted(bl, key=lambda p: (p % 8, p // 8))]
    return out

def issue_list(order, pattern=(1, 1, 0, 0), lag=27, shift=True, fuse=False):
    P = len(pattern); n = len(order)
    pr = [pattern[i % P] if i < n - lag else 1 for i in range(n)]
    if not shift:
        pr = [pattern[(i - lag) % P] if i >= lag else 1 for i in range(n)]
    ds_ = []
    for i, x in enumerate(order):
        if fuse and ds_ and len(ds_[-1][0]) == 1 and ds_[-1][1] == pr[i]:
            t0, p0 = ds_[-1][0][0]
            if x[0] == t0 and t0 in ("k", "v", "wq", "wo") and x[1] - p0 == (64 if t0 in "kv" else 32):
                ds_[-1][0].append(x); continue
        ds_.append([[x], pr[i]])
    ds_ = [(xs, p, i) for i, (xs, p) in enumerate(ds_)]
    if not shift:
        return [(xs, p, e + (lag if p else -lag)) for xs, p, e in ds_]
    p1 = [d for d in ds_ if d[1] == 1]; p0 = [d for d in ds_ if d[1] == 0]
    out = p1[:lag]; i0, i1 = 0, lag
    for d in ds_:
        if d[1] == 1:
            if i1 < len(p1): out.append(p1[i1]); i1 += 1
        else: out.append(p0[i0]); i0 += 1
    assert len(out) == len(ds_)
    return out

def make(order, w2_stages, name="k", ahead=62, gaps=None, skip=(), lag=27, pattern=(1, 1, 0, 0), vpu=(), flags=None,
         shift=True, fuse=False, ck=512, late=None):
    issue = issue_list(order, pattern, lag, shift, fuse)
    gaps = dict(dict(wq=16, kv=32, wo=10, w1=0, w2=0), **(gaps or {}))
    p2stage = {p: i for i, bl in enumerate(w2_stages) for p in bl}
    ppc = ck // 64; nch = 4096 // ck
    def stage_of(x):
        t, p = x
        if t == "w2": return (t, p2stage[p])
        if t in "kv": return ("kv", p % 64 // ppc)
        if t == "wq": return (t, p % 4)
        if t == "wo": return (t, p % 32 // 8)
        return (t, 0)
    last = {}
    for i, (xs, pr, e) in enumerate(issue):
        last[stage_of(xs[0])] = max(last.get(stage_of(xs[0]), 0), e + lag, i)
    semid = {s: i + 3 for i, s in enumerate(last)}
    def fn(x, k, v, wq, wo, bx, w1, b1, w2, b2):
        _, hkv, sk, dh = k.shape
        d = x.shape[-1]; f = w1.shape[1]
        win = min(4096, max(256, sk // 4)); s0 = sk - win
        def kern(x_h, k_h, v_h, wq_h, wo_h, w1_h, b1_h, w2_h, b2_h, o_ref,
                 xb, kvb, wqb, wob, w1b, b1b, w2b, b2b, sems):
            ds = pl.ds
            slot = {p: i for i, p in enumerate(p for bl in w2_stages for p in bl)}
            def start(xs, pr, e):
                t, p = xs[0]; m = len(xs)
                sem = sems.at[semid[stage_of(xs[0])]]
                if t in "kv":
                    s_ = k_h if t == "k" else v_h
                    j = p % 64
                    cps = [(s_.at[0, ds(p // 64, m), ds(s0 + j * 64, 64)], kvb.at[j // ppc, int(t == "v"), ds(p // 64, m), ds(j % ppc * 64, 64)])]
                elif t == "wq":
                    cps = [(wq_h.at[ds(p // 32, m), ds(p % 32 // 4 * 8, 8), ds(p % 4 * 1024, 1024)], wqb.at[p % 4, ds(p // 32, m), ds(p % 32 // 4 * 8, 8)])]
                elif t == "wo":
                    cps = [(wo_h.at[ds(p // 32, m), ds(p % 32 * 16, 16)], wob.at[p % 32 // 8, ds(p // 32, m), ds(p % 8 * 16, 16)])]
                elif t == "w2":
                    cps = [(w2_h.at[ds(p * 16, 16)], w2b.at[ds(slot[p] * 16, 16)])]
                else:
                    cps = []; a, b = 8 * p, 8 * p + 8
                    while a < b:
                        rg, ct = divmod(a, 14); n = min(b - a, 14 - ct)
                        ix = (ds(rg * 8, 8), ds(ct * 128, n * 128)); cps.append((w1_h.at[ix], w1b.at[ix])); a += n
                for s_, d_ in cps:
                    pltpu.make_async_copy(s_, d_, sem).start(priority=pr)
            pos = [0]; prev = [0]
            def upto(n):
                n = min(n, len(issue))
                while pos[0] < n:
                    start(*issue[pos[0]]); pos[0] += 1
            def wait(stage, buf):
                ah = ahead if (late is None or stage[0] in ("wq", "kv")) else late
                upto(max(last[stage] + 1 + ah, pos[0] + prev[0])); prev[0] = gaps[stage[0]]
                pltpu.make_async_copy(buf, buf, sems.at[semid[stage]]).wait()
            small = [pltpu.make_async_copy(s_, d_, sems.at[i]) for i, (s_, d_) in enumerate(((x_h, xb), (b1_h, b1b), (b2_h, b2b)))]
            upto(8)
            for c in small: c.start()
            upto(100)
            for c in small: c.wait()
            x8 = jnp.broadcast_to(xb[0].astype(F32), (8, d))
            xn = _ln(x8).astype(BF16)
            row = lax.broadcasted_iota(jnp.int32, (8, dh), 0)
            nt = (((1,), (1,)), ((), ()))
            qs = []
            for a in range(4):
                wait(("wq", a), wqb.at[a])
                if "q" in skip:
                    qs.append(xn[:, :128]); continue
                q = jnp.dot(xn, wqb[a].reshape(512, 1024), preferred_element_type=F32)
                qa = q[:, :dh]
                for r in range(1, 8):
                    qa = jnp.where(row == r, q[:, r * dh:(r + 1) * dh], qa)
                qs.append(qa.astype(BF16))
            st = [None] * 4
            for c in range(nch):
                wait(("kv", c), kvb.at[c])
                if "k" in skip: continue
                for a in range(4):
                    s_lo = lax.dot_general(qs[a], kvb[c, 0, 2 * a], nt, preferred_element_type=F32)
                    s_hi = lax.dot_general(qs[a], kvb[c, 0, 2 * a + 1], nt, preferred_element_type=F32)
                    s = jnp.where(row[:, :1] < 4, s_lo, s_hi) * (dh ** -0.5)
                    m = jnp.max(s, axis=-1, keepdims=True)
                    if c: m = jnp.maximum(m, st[a][0])
                    e = jnp.exp(s - m)
                    l = jnp.sum(e, axis=-1, keepdims=True)
                    eb = e.astype(BF16)
                    o = jnp.where(row < 4, jnp.dot(eb, kvb[c, 1, 2 * a], preferred_element_type=F32),
                                  jnp.dot(eb, kvb[c, 1, 2 * a + 1], preferred_element_type=F32))
                    if c:
                        al = jnp.exp(st[a][0] - m)
                        l = l + al * st[a][1]; o = o + al * st[a][2]
                    st[a] = (m, l, o)
            os_ = [qs[a].astype(F32) if "k" in skip else st[a][2] / st[a][1] for a in range(4)]
            acc = jnp.zeros((8, d), F32)
            for c in range(4):
                lhs = jnp.concatenate([jnp.where(row == (s % 2) * 4 + c, os_[s // 2], 0.0) for s in range(8)], axis=1).astype(BF16)
                wait(("wo", c), wob.at[c])
                if "o" in skip:
                    acc = acc + lhs[:, :512].astype(F32); continue
                acc = acc + jnp.dot(lhs, wob[c].reshape(1024, 512), preferred_element_type=F32)
            h = x8 + jnp.sum(acc, axis=0, keepdims=True)
            y = _ln(_ln(h)).astype(BF16)
            wait(("w1", 0), w1b)
            upto(len(issue))
            if "1" in skip:
                g = jnp.concatenate([y] * 4, axis=1).astype(F32)
            else:
                z = jnp.dot(y, w1b[...], preferred_element_type=F32) + b1b[...].astype(F32).reshape(1, f)
                g = jax.nn.gelu(z, approximate=True)
            out = h + b2b[...].astype(F32).reshape(1, d)
            gT = {}
            for i in vpu:
                for p in w2_stages[i]:
                    b = p // 8
                    if b not in gT:
                        gb = g[:, 128 * b:128 * b + 128].astype(BF16).astype(F32)
                        gT[b] = jnp.broadcast_to(gb[0:1], (128, 128)).T
            part = None
            for i, bl in enumerate(w2_stages):
                r0 = slot[bl[0]] * 16; n = 16 * len(bl)
                if i not in vpu:
                    runs = []
                    for p in bl:
                        if runs and runs[-1][1] == 16 * p: runs[-1][1] += 16
                        else: runs.append([16 * p, 16 * p + 16])
                    gl = jnp.concatenate([g[:, a:b] for a, b in runs], axis=1).astype(BF16)
                wait(("w2", i), w2b.at[ds(r0, n)])
                if "2" in skip: continue
                if i not in vpu:
                    out = out + jnp.dot(gl, w2b[ds(r0, n), :], preferred_element_type=F32)
                else:
                    for p in bl:
                        gc = gT[p // 8][p % 8 * 16:p % 8 * 16 + 16]
                        pr = w2b[ds(slot[p] * 16, 16), :].astype(F32) * jnp.concatenate([gc] * 4, axis=1)
                        pr = pr[:8] + pr[8:]
                        part = pr if part is None else part + pr
            if part is not None:
                o_ref[0] = (out[0:1] + jnp.sum(part, axis=0, keepdims=True)).astype(o_ref.dtype)
            else:
                o_ref[0] = out[0:1].astype(o_ref.dtype)
        hbm = pl.BlockSpec(memory_space=pltpu.HBM)
        V = pltpu.VMEM
        return pl.pallas_call(
            kern, out_shape=jax.ShapeDtypeStruct(x.shape, x.dtype), in_specs=[hbm] * 9,
            scratch_shapes=[V(x.shape, x.dtype), V((nch, 2, hkv, ck, dh), k.dtype), V((4, 8, 64, 1024), wq.dtype),
                            V((4, 8, 128, 512), wo.dtype), V(w1.shape, w1.dtype), V(b1.shape, b1.dtype), V(w2.shape, w2.dtype),
                            V(b2.shape, b2.dtype), pltpu.SemaphoreType.DMA((3 + len(semid),))],
            compiler_params=pltpu.CompilerParams(vmem_limit_bytes=48 * 2**20, disable_bounds_checks=True, disable_semaphore_checks=True, flags=flags),
            name=name)(x, k, v, wq.reshape(8, 64, 4096), wo.reshape(8, 512, 512), w1, b1, w2, b2)
    return fn

def taper(o=96, a=104, b=116): return build_order(grp("wq", 0), grp("k", 32), grp("v", 32), grp("wo", o), grp("w1", a), grp("w2", b))
T3 = [blk(0, 4, 8, 12, 1, 5, 9, 13, 2, 6, 10), blk(3, 7), blk(11)]
T4 = [blk(0, 4, 8, 12, 1, 5, 9, 13), blk(2, 6, 10), blk(3, 7), blk(11)]


_fn = make(with_tail(taper(96, 104, 124), T4, 2), T4, "decode_block", vpu=(3,), fuse=True)


@jax.jit
def pallas_sequential_preLN__sliding_block_cached__mixer_channel_mlp__decode_kernel(
    A_x, A_k_cache, A_v_cache, A_wq, A_wo, B_x, B_w1, B_b1, B_w2, B_b2):
    return _fn(A_x, A_k_cache, A_v_cache, A_wq, A_wo, B_x, B_w1, B_b1, B_w2, B_b2)
```

```python
import jax
import jax.experimental.pallas as pl
import jax.experimental.pallas.tpu as pltpu
import jax.numpy as jnp
from jax import lax

_F32 = jnp.float32
_LANES = 128
_SUBLANES = 8

_PIECE = 8192
_ROUNDS = 32
_KEY_CHUNK = 512
_QUEUE_DEPTH = 24
_EARLY = (6, 18)
_AHEAD = 62
_W1_FIRST_ROUND = 4
_W2_FIRST_ROUND = 28

_KV_VISIT = (0, 1, 10, 11, 14, 15, 4, 5, 8, 9, 2, 3, 6, 7, 12, 13)
_W_VISIT = (0, 4, 2, 6, 1, 5, 3, 7)


class _Stream:
    def __init__(self, pieces, tail, sems):
        arrival = [(c, 1 - i // 2 % 2) for i, piece in enumerate(pieces) for c in piece]
        arrival += [(c, 1) for piece in tail for c in piece]
        queues = [iter([c for c, priority in arrival if priority == p]) for p in (0, 1)]
        steady = [priority for _, priority in arrival[:-_QUEUE_DEPTH]]
        fill = [1] * _QUEUE_DEPTH
        for at in _EARLY:
            fill.insert(at, steady.pop(steady.index(0)))
        self._order = [(next(queues[p]), p) for p in fill + steady]
        self._due = {c[2]: i + _QUEUE_DEPTH + 1 for i, (c, _) in enumerate(arrival)}
        self._sems = {stage: sems.at[i] for i, stage in enumerate(self._due)}
        self._started = 0

    def wait(self, stage, slab, refill=0):
        until = max(self._due[stage] + _AHEAD, self._started + refill)
        for (src, dst, s), priority in self._order[self._started:until]:
            pltpu.make_async_copy(src, dst, self._sems[s]).start(priority=priority)
        self._started = until
        pltpu.make_async_copy(slab, slab, self._sems[stage]).wait()


def _layernorm(x):
    inv_n = 1.0 / x.shape[-1]
    centered = x - jnp.sum(x, axis=-1, keepdims=True) * inv_n
    var = jnp.sum(centered * centered, axis=-1, keepdims=True) * inv_n
    return centered * lax.rsqrt(var + 1e-5)


def _dot(a, b):
    return jnp.dot(a, b, preferred_element_type=_F32)


def _dot_nt(a, b):
    return lax.dot_general(a, b, (((1,), (1,)), ((), ())), preferred_element_type=_F32)


def _w2_blocks(d_ff):
    blocks = range(d_ff // _LANES)
    return tuple([b for b in blocks if b % 4 in phases] for phases in ((0, 1), (2,), (3,)))


def _kernel(x_hbm, k_hbm, v_hbm, wq_hbm, wo_hbm, w1_hbm, b1_hbm, w2_hbm, b2_hbm, o_ref,
            kv_buf, wq_buf, wo_buf, w1_buf, w2_buf, x_buf, b1_buf, b2_buf, sems):
    n_chunks, _, kv_heads, _, d_head = kv_buf.shape
    d_model, d_ff = w1_buf.shape
    n_packs = kv_heads // 2
    group = _SUBLANES // 2
    window = n_chunks * _KEY_CHUNK
    first_key = k_hbm.shape[2] - window
    keys, rows = _PIECE // d_head, _PIECE // d_model
    mxu_a, mxu_b, vpu = _w2_blocks(d_ff)
    w2_slot = {b: i * _LANES for i, b in enumerate(mxu_a + mxu_b + vpu)}

    def wq_piece(p):
        row, pack = divmod(p, n_packs)
        tile_row, width = pl.ds(row * _SUBLANES, _SUBLANES), wq_buf.shape[2]
        return [(wq_hbm.at[tile_row, pl.ds(pack * width, width)], wq_buf.at[pack, tile_row],
                 ("wq", pack))]

    def kv_piece(key, cache, head):
        chunk, at = divmod(key, _KEY_CHUNK)
        return [((k_hbm, v_hbm)[cache].at[0, head, pl.ds(first_key + key, keys)],
                 kv_buf.at[chunk, cache, head, pl.ds(at, keys)], ("kv", chunk))]

    def wo_piece(p):
        head, at = divmod(p * rows, d_head)
        return [(wo_hbm.at[pl.ds(p * rows, rows)],
                 wo_buf.at[head % group, pl.ds(head // group * d_head + at, rows)],
                 ("wo", head % group))]

    def w1_piece(p):
        row, col = divmod(p * 8, d_ff // _LANES)
        n = min(8, d_ff // _LANES - col)
        spans = [(row, col, n)] + ([(row + 1, 0, 8 - n)] if n < 8 else [])
        views = [(pl.ds(r * _SUBLANES, _SUBLANES), pl.ds(c * _LANES, m * _LANES))
                 for r, c, m in spans]
        return [(w1_hbm.at[view], w1_buf.at[view], "w1") for view in views]

    def w2_piece(p):
        block, at = divmod(p * rows, _LANES)
        stage = "w2a" if block in mxu_a else "w2b" if block in mxu_b else ("w2", p)
        return [(w2_hbm.at[pl.ds(p * rows, rows)],
                 w2_buf.at[pl.ds(w2_slot[block] + at, rows)], stage)]

    mlp_pieces = d_model * d_ff // _PIECE
    vpu_pieces = [p for p in range(mlp_pieces) if p * rows // _LANES in vpu]
    small = [(x_hbm, x_buf, "x"), (b1_hbm, b1_buf, "b1"), (b2_hbm, b2_buf, "b2")]
    pieces = [wq_piece(s * _ROUNDS + r) for r in range(_ROUNDS) for s in _W_VISIT]
    pieces[3] += small
    pieces += [kv_piece(key, *divmod(s, kv_heads))
               for key in range(0, window, keys) for s in _KV_VISIT]
    for r in range(_W2_FIRST_ROUND + _ROUNDS):
        if r < _ROUNDS:
            pieces += [wo_piece(s * _ROUNDS + r) for s in _W_VISIT]
        if 0 <= r - _W1_FIRST_ROUND < _ROUNDS:
            pieces += [w1_piece(p) for p in range(r - _W1_FIRST_ROUND, mlp_pieces, _ROUNDS)]
        if 0 <= r - _W2_FIRST_ROUND:
            pieces += [w2_piece(p) for p in range(r - _W2_FIRST_ROUND, mlp_pieces, _ROUNDS)
                       if p not in vpu_pieces]
    stream = _Stream(pieces, [w2_piece(p) for p in vpu_pieces], sems)

    for _, buf, stage in small:
        stream.wait(stage, buf)
    x = jnp.broadcast_to(x_buf[0].astype(_F32), (_SUBLANES, d_model))
    xn = _layernorm(x).astype(wq_buf.dtype)
    sublane = lax.broadcasted_iota(jnp.int32, (_SUBLANES, 1), 0)
    q = []
    for pack in range(n_packs):
        stream.wait(("wq", pack), wq_buf.at[pack], refill=16)
        flat = _dot(xn, wq_buf[pack])
        heads = flat[:, :d_head]
        for i in range(1, _SUBLANES):
            heads = jnp.where(sublane == i, flat[:, i * d_head:(i + 1) * d_head], heads)
        q.append(heads.astype(kv_buf.dtype))

    def per_kv_head(product, lhs, chunk, cache, pack):
        return jnp.where(sublane < group, product(lhs, kv_buf[chunk, cache, 2 * pack]),
                         product(lhs, kv_buf[chunk, cache, 2 * pack + 1]))

    row_max, denom, numer = [None] * n_packs, [None] * n_packs, [None] * n_packs
    for chunk in range(n_chunks):
        stream.wait(("kv", chunk), kv_buf.at[chunk], refill=16)
        scores = [per_kv_head(_dot_nt, q[pack], chunk, 0, pack) * d_head ** -0.5
                  for pack in range(n_packs)]
        new_max = [jnp.max(s, axis=-1, keepdims=True) for s in scores]
        if chunk:
            new_max = [jnp.maximum(a, b) for a, b in zip(new_max, row_max)]
        weights = [jnp.exp(s - m) for s, m in zip(scores, new_max)]
        for pack, w in enumerate(weights):
            den = sum(w[:, i:i + _LANES] for i in range(0, _KEY_CHUNK, _LANES))
            num = per_kv_head(_dot, w.astype(kv_buf.dtype), chunk, 1, pack)
            if chunk:
                decay = jnp.exp(row_max[pack] - new_max[pack])
                den, num = den + decay * denom[pack], num + decay * numer[pack]
            denom[pack], numer[pack] = den, num
        row_max = new_max
    attn = [n / jnp.sum(d, axis=-1, keepdims=True) for n, d in zip(numer, denom)]

    proj = 0.0
    for q_head in range(group):
        lhs = jnp.concatenate(
            [jnp.where(sublane == kv % 2 * group + q_head, attn[kv // 2], 0.0)
             for kv in range(kv_heads)], axis=1).astype(wo_buf.dtype)
        stream.wait(("wo", q_head), wo_buf.at[q_head], refill=10)
        proj = proj + _dot(lhs, wo_buf[q_head])
    h = x + jnp.sum(proj, axis=0, keepdims=True)

    y = _layernorm(_layernorm(h)).astype(w1_buf.dtype)
    stream.wait("w1", w1_buf)
    hidden = _dot(y, w1_buf[...]) + b1_buf[...].astype(_F32).reshape(1, d_ff)
    hidden = jax.nn.gelu(hidden, approximate=True)
    hidden = [hidden[:, i:i + _LANES] for i in range(0, d_ff, _LANES)]
    column = {b: jnp.broadcast_to(hidden[b][:1], (_LANES, _LANES)).T for b in vpu}

    out = h + b2_buf[...].astype(_F32).reshape(1, d_model)
    for stage, blocks in (("w2a", mxu_a), ("w2b", mxu_b)):
        lhs = jnp.concatenate([hidden[b] for b in blocks], axis=1).astype(w2_buf.dtype)
        slab = pl.ds(w2_slot[blocks[0]], len(blocks) * _LANES)
        stream.wait(stage, w2_buf.at[slab])
        out = out + _dot(lhs, w2_buf[slab])
    out = jnp.where(sublane == 0, out, 0.0)
    for p in vpu_pieces:
        block, at = divmod(p * rows, _LANES)
        scale = jnp.concatenate([column[block][at:at + rows]] * (d_model // _LANES), axis=1)
        slab = pl.ds(w2_slot[block] + at, rows)
        stream.wait(("w2", p), w2_buf.at[slab])
        terms = w2_buf[slab].astype(_F32) * scale
        for i in range(0, rows, _SUBLANES):
            out = out + terms[i:i + _SUBLANES]
    o_ref[0] = jnp.sum(out, axis=0, keepdims=True).astype(o_ref.dtype)


@jax.jit
def pallas_sequential_preLN__sliding_block_cached__mixer_channel_mlp__decode_kernel(
    A_x: jax.Array,
    A_k_cache: jax.Array,
    A_v_cache: jax.Array,
    A_wq: jax.Array,
    A_wo: jax.Array,
    B_x: jax.Array,
    B_w1: jax.Array,
    B_b1: jax.Array,
    B_w2: jax.Array,
    B_b2: jax.Array,
):
    del B_x
    _, kv_heads, cache_len, d_head = A_k_cache.shape
    d_model, d_attn = A_wq.shape
    d_ff = B_w1.shape[1]
    window = min(4096, max(256, cache_len // 4))
    assert A_x.shape == (1, 1, 512) and (kv_heads, d_head, d_attn) == (8, 128, 4096)
    assert window % _KEY_CHUNK == 0 and d_ff % _LANES == 0
    n_chunks = window // _KEY_CHUNK
    n_stages = 3 + 4 + n_chunks + 4 + 3 + len(_w2_blocks(d_ff)[2]) * _LANES * d_model // _PIECE

    return pl.pallas_call(
        _kernel,
        out_shape=jax.ShapeDtypeStruct(A_x.shape, A_x.dtype),
        in_specs=[pl.BlockSpec(memory_space=pltpu.HBM)] * 9,
        scratch_shapes=[
            pltpu.VMEM((n_chunks, 2, kv_heads, _KEY_CHUNK, d_head), A_k_cache.dtype),
            pltpu.VMEM((4, d_model, d_attn // 4), A_wq.dtype),
            pltpu.VMEM((4, d_attn // 4, d_model), A_wo.dtype),
            pltpu.VMEM(B_w1.shape, B_w1.dtype),
            pltpu.VMEM(B_w2.shape, B_w2.dtype),
            pltpu.VMEM(A_x.shape, A_x.dtype),
            pltpu.VMEM(B_b1.shape, B_b1.dtype),
            pltpu.VMEM(B_b2.shape, B_b2.dtype),
            pltpu.SemaphoreType.DMA((n_stages,)),
        ],
        compiler_params=pltpu.CompilerParams(
            vmem_limit_bytes=40 * 1024 * 1024,
            disable_semaphore_checks=True,
        ),
        name="decode_block",
    )(A_x, A_k_cache, A_v_cache, A_wq, A_wo, B_w1, B_b1, B_w2, B_b2)
```

```python
import jax
import jax.experimental.pallas as pl
import jax.experimental.pallas.tpu as pltpu
import jax.numpy as jnp
from jax import lax

_F32 = jnp.float32
_LANES = 128
_SUBLANES = 8

_PIECE = 8192
_ROUNDS = 32
_KEY_CHUNK = 512
_QUEUE_DEPTH = 24
_EARLY = (6, 18)
_AHEAD = 62
_W1_FIRST_ROUND = 4
_W2_FIRST_ROUND = 28

_KV_VISIT = (0, 1, 10, 11, 14, 15, 4, 5, 8, 9, 2, 3, 6, 7, 12, 13)
_W_VISIT = (0, 4, 2, 6, 1, 5, 3, 7)


class _Stream:
    def __init__(self, pieces, tail, sems):
        arrival = [(c, 1 - i // 2 % 2) for i, piece in enumerate(pieces) for c in piece]
        arrival += [(c, 1) for piece in tail for c in piece]
        queues = [iter([c for c, priority in arrival if priority == p]) for p in (0, 1)]
        steady = [priority for _, priority in arrival[:-_QUEUE_DEPTH]]
        fill = [1] * _QUEUE_DEPTH
        for at in _EARLY:
            fill.insert(at, steady.pop(steady.index(0)))
        self._order = [(next(queues[p]), p) for p in fill + steady]
        self._due = {c[2]: i + _QUEUE_DEPTH + 1 for i, (c, _) in enumerate(arrival)}
        self._sems = {stage: sems.at[i] for i, stage in enumerate(self._due)}
        self._started = 0

    def wait(self, stage, slab, refill=0):
        until = max(self._due[stage] + _AHEAD, self._started + refill)
        for (src, dst, s), priority in self._order[self._started:until]:
            pltpu.make_async_copy(src, dst, self._sems[s]).start(priority=priority)
        self._started = until
        assert all(s != stage for (_, _, s), _ in self._order[until:])
        pltpu.make_async_copy(slab, slab, self._sems[stage]).wait()


def _layernorm(x):
    inv_n = 1.0 / x.shape[-1]
    centered = x - jnp.sum(x, axis=-1, keepdims=True) * inv_n
    var = jnp.sum(centered * centered, axis=-1, keepdims=True) * inv_n
    return centered * lax.rsqrt(var + 1e-5)


def _dot(a, b):
    return jnp.dot(a, b, preferred_element_type=_F32)


def _dot_nt(a, b):
    return lax.dot_general(a, b, (((1,), (1,)), ((), ())), preferred_element_type=_F32)


def _w2_blocks(d_ff):
    blocks = range(d_ff // _LANES)
    return tuple([b for b in blocks if b % 4 in phases] for phases in ((0, 1), (2,), (3,)))


def _kernel(x_hbm, k_hbm, v_hbm, wq_hbm, wo_hbm, w1_hbm, b1_hbm, w2_hbm, b2_hbm, o_ref,
            kv_buf, wq_buf, wo_buf, w1_buf, w2_buf, x_buf, b1_buf, b2_buf, sems):
    n_chunks, _, kv_heads, _, d_head = kv_buf.shape
    d_model, d_ff = w1_hbm.shape
    n_packs = kv_heads // 2
    group = _SUBLANES // 2
    window = n_chunks * _KEY_CHUNK
    first_key = k_hbm.shape[2] - window
    keys, rows = _PIECE // d_head, _PIECE // d_model
    mxu_a, mxu_b, vpu = _w2_blocks(d_ff)
    w2_slot = {b: i * _LANES for i, b in enumerate(mxu_a + mxu_b + vpu)}

    def wq_piece(p):
        row, pack = divmod(p, n_packs)
        tile_row, width = pl.ds(row * _SUBLANES, _SUBLANES), wq_buf.shape[3]
        return [(wq_hbm.at[tile_row, pl.ds(pack * width, width)], wq_buf.at[pack, row],
                 ("wq", pack))]

    def kv_piece(key, cache, head):
        chunk, at = divmod(key, _KEY_CHUNK)
        return [((k_hbm, v_hbm)[cache].at[0, head, pl.ds(first_key + key, keys)],
                 kv_buf.at[chunk, cache, head, pl.ds(at, keys)], ("kv", chunk))]

    def wo_piece(p):
        head, at = divmod(p * rows, d_head)
        return [(wo_hbm.at[pl.ds(p * rows, rows)],
                 wo_buf.at[head % group, pl.ds(head // group * d_head + at, rows)],
                 ("wo", head % group))]

    def w1_piece(p):
        row, col = divmod(p * 8, d_ff // _LANES)
        n = min(8, d_ff // _LANES - col)
        spans = [(row, col, n)] + ([(row + 1, 0, 8 - n)] if n < 8 else [])
        return [(w1_hbm.at[pl.ds(r * _SUBLANES, _SUBLANES), pl.ds(c * _LANES, m * _LANES)],
                 w1_buf.at[r, :, pl.ds(c * _LANES, m * _LANES)], "w1") for r, c, m in spans]

    def w2_piece(p):
        block, at = divmod(p * rows, _LANES)
        stage = "w2a" if block in mxu_a else "w2b" if block in mxu_b else ("w2", p)
        return [(w2_hbm.at[pl.ds(p * rows, rows)],
                 w2_buf.at[pl.ds(w2_slot[block] + at, rows)], stage)]

    mlp_pieces = d_model * d_ff // _PIECE
    vpu_pieces = [p for p in range(mlp_pieces) if p * rows // _LANES in vpu]
    small = [(x_hbm, x_buf, "x"), (b1_hbm, b1_buf, "b1"), (b2_hbm, b2_buf, "b2")]
    pieces = [wq_piece(s * _ROUNDS + r) for r in range(_ROUNDS) for s in _W_VISIT]
    pieces[3] += small
    pieces += [kv_piece(key, *divmod(s, kv_heads))
               for key in range(0, window, keys) for s in _KV_VISIT]
    for r in range(_W2_FIRST_ROUND + _ROUNDS):
        if r < _ROUNDS:
            pieces += [wo_piece(s * _ROUNDS + r) for s in _W_VISIT]
        if 0 <= r - _W1_FIRST_ROUND < _ROUNDS:
            pieces += [w1_piece(p) for p in range(r - _W1_FIRST_ROUND, mlp_pieces, _ROUNDS)]
        if 0 <= r - _W2_FIRST_ROUND:
            pieces += [w2_piece(p) for p in range(r - _W2_FIRST_ROUND, mlp_pieces, _ROUNDS)
                       if p not in vpu_pieces]
    stream = _Stream(pieces, [w2_piece(p) for p in vpu_pieces], sems)

    for _, buf, stage in small:
        stream.wait(stage, buf)
    x = jnp.broadcast_to(x_buf[0].astype(_F32), (_SUBLANES, d_model))
    xn = _layernorm(x).astype(wq_buf.dtype)
    sublane = lax.broadcasted_iota(jnp.int32, (_SUBLANES, 1), 0)
    q = []
    for pack in range(n_packs):
        stream.wait(("wq", pack), wq_buf.at[pack], refill=16)
        flat = _dot(xn, wq_buf[pack].reshape(d_model, -1))
        heads = flat[:, :d_head]
        for i in range(1, _SUBLANES):
            heads = jnp.where(sublane == i, flat[:, i * d_head:(i + 1) * d_head], heads)
        q.append(heads.astype(kv_buf.dtype))

    def per_kv_head(product, lhs, chunk, cache, pack):
        return jnp.where(sublane < group, product(lhs, kv_buf[chunk, cache, 2 * pack]),
                         product(lhs, kv_buf[chunk, cache, 2 * pack + 1]))

    row_max, denom, numer = [None] * n_packs, [None] * n_packs, [None] * n_packs
    for chunk in range(n_chunks):
        stream.wait(("kv", chunk), kv_buf.at[chunk], refill=16)
        scores = [per_kv_head(_dot_nt, q[pack], chunk, 0, pack) * d_head ** -0.5
                  for pack in range(n_packs)]
        new_max = [jnp.max(s, axis=-1, keepdims=True) for s in scores]
        if chunk:
            new_max = [jnp.maximum(a, b) for a, b in zip(new_max, row_max)]
        weights = [jnp.exp(s - m) for s, m in zip(scores, new_max)]
        for pack, w in enumerate(weights):
            den = sum(w[:, i:i + _LANES] for i in range(0, _KEY_CHUNK, _LANES))
            num = per_kv_head(_dot, w.astype(kv_buf.dtype), chunk, 1, pack)
            if chunk:
                decay = jnp.exp(row_max[pack] - new_max[pack])
                den, num = den + decay * denom[pack], num + decay * numer[pack]
            denom[pack], numer[pack] = den, num
        row_max = new_max
    attn = [n / jnp.sum(d, axis=-1, keepdims=True) for n, d in zip(numer, denom)]

    proj = 0.0
    for q_head in range(group):
        lhs = jnp.concatenate(
            [jnp.where(sublane == kv % 2 * group + q_head, attn[kv // 2], 0.0)
             for kv in range(kv_heads)], axis=1).astype(wo_buf.dtype)
        stream.wait(("wo", q_head), wo_buf.at[q_head], refill=10)
        proj = proj + _dot(lhs, wo_buf[q_head])
    h = x + jnp.sum(proj, axis=0, keepdims=True)

    y = _layernorm(_layernorm(h)).astype(w1_buf.dtype)
    stream.wait("w1", w1_buf)
    hidden = _dot(y, w1_buf[...].reshape(d_model, d_ff))
    hidden = jax.nn.gelu(hidden + b1_buf[...].astype(_F32).reshape(1, d_ff), approximate=True)
    hidden = [hidden[:, i:i + _LANES] for i in range(0, d_ff, _LANES)]
    column = {b: jnp.broadcast_to(hidden[b][:1], (_LANES, _LANES)).T for b in vpu}

    out = h + b2_buf[...].astype(_F32).reshape(1, d_model)
    for stage, blocks in (("w2a", mxu_a), ("w2b", mxu_b)):
        lhs = jnp.concatenate([hidden[b] for b in blocks], axis=1).astype(w2_buf.dtype)
        slab = pl.ds(w2_slot[blocks[0]], len(blocks) * _LANES)
        stream.wait(stage, w2_buf.at[slab])
        out = out + _dot(lhs, w2_buf[slab])
    out = jnp.where(sublane == 0, out, 0.0)
    for p in vpu_pieces:
        block, at = divmod(p * rows, _LANES)
        scale = jnp.concatenate([column[block][at:at + rows]] * (d_model // _LANES), axis=1)
        slab = pl.ds(w2_slot[block] + at, rows)
        stream.wait(("w2", p), w2_buf.at[slab])
        terms = w2_buf[slab].astype(_F32) * scale
        for i in range(0, rows, _SUBLANES):
            out = out + terms[i:i + _SUBLANES]
    o_ref[0] = jnp.sum(out, axis=0, keepdims=True).astype(o_ref.dtype)


@jax.jit
def pallas_sequential_preLN__sliding_block_cached__mixer_channel_mlp__decode_kernel(
    A_x: jax.Array,
    A_k_cache: jax.Array,
    A_v_cache: jax.Array,
    A_wq: jax.Array,
    A_wo: jax.Array,
    B_x: jax.Array,
    B_w1: jax.Array,
    B_b1: jax.Array,
    B_w2: jax.Array,
    B_b2: jax.Array,
):
    del B_x
    _, kv_heads, cache_len, d_head = A_k_cache.shape
    d_model, d_attn = A_wq.shape
    d_ff = B_w1.shape[1]
    window = min(4096, max(256, cache_len // 4))
    assert A_x.shape == (1, 1, 512) and (kv_heads, d_head, d_attn) == (8, 128, 4096)
    assert window % _KEY_CHUNK == 0 and d_ff % _LANES == 0
    n_chunks = window // _KEY_CHUNK
    vpu_pieces = len(_w2_blocks(d_ff)[2]) * _LANES * d_model // _PIECE
    n_stages = 3 + 4 + n_chunks + 4 + 1 + 2 + vpu_pieces

    return pl.pallas_call(
        _kernel,
        out_shape=jax.ShapeDtypeStruct(A_x.shape, A_x.dtype),
        in_specs=[pl.BlockSpec(memory_space=pltpu.HBM)] * 9,
        scratch_shapes=[
            pltpu.VMEM((n_chunks, 2, kv_heads, _KEY_CHUNK, d_head), A_k_cache.dtype),
            pltpu.VMEM((4, d_model // _SUBLANES, _SUBLANES, d_attn // 4), A_wq.dtype),
            pltpu.VMEM((4, d_attn // 4, d_model), A_wo.dtype),
            pltpu.VMEM((d_model // _SUBLANES, _SUBLANES, d_ff), B_w1.dtype),
            pltpu.VMEM(B_w2.shape, B_w2.dtype),
            pltpu.VMEM(A_x.shape, A_x.dtype),
            pltpu.VMEM(B_b1.shape, B_b1.dtype),
            pltpu.VMEM(B_b2.shape, B_b2.dtype),
            pltpu.SemaphoreType.DMA((n_stages,)),
        ],
        compiler_params=pltpu.CompilerParams(
            vmem_limit_bytes=40 * 1024 * 1024,
            disable_semaphore_checks=True,
        ),
        name="decode_block",
    )(A_x, A_k_cache, A_v_cache, A_wq, A_wo, B_w1, B_b1, B_w2, B_b2)
```
